```python
import os as _os
_os.environ.setdefault("JAX_PLATFORMS", "cpu")
import jax
import jax.numpy as jnp

def _softmax(x, axis=-1):
    return jax.nn.softmax(x, axis=axis)
def _gelu(x):
    return jax.nn.gelu(x, approximate=True)
def _silu(x):
    return jax.nn.silu(x)
def _sigmoid(x):
    return jax.nn.sigmoid(x)
def _layernorm(x, axis=-1, eps=1e-5):
    m = jnp.mean(x, axis=axis, keepdims=True)
    v = jnp.var(x, axis=axis, keepdims=True)
    return (x - m) / jnp.sqrt(v + eps)
def _scatter_add(tgt, idx, src, axis=0):
    return tgt.at[idx].add(src)
def _segment_sum(src, seg, n):
    return jax.ops.segment_sum(src, seg, n)
class _Rng:
    def __init__(self, key):
        self._k = key
    def _next(self):
        self._k, sub = jax.random.split(self._k)
        return sub
    def normal(self, shape):
        return jax.random.normal(self._next(), shape, dtype=jnp.bfloat16)
    def randint(self, lo, hi, shape):
        return jax.random.randint(self._next(), shape, lo, hi, dtype=jnp.int32)
    def uniform(self, shape, lo=0.0, hi=1.0):
        return jax.random.uniform(self._next(), shape, jnp.bfloat16, lo, hi)
    def permutation(self, n):
        return jax.random.permutation(self._next(), n)


kernel_name = 'standalone__gqa_block_cached__near_ridge'

def setup_inputs():
    _rng = _Rng(jax.random.key(int.from_bytes(__import__("os").urandom(4), "little")))
    _w = (lambda a: (lambda t: t.astype(jnp.bfloat16) if jnp.issubdtype(t.dtype, jnp.floating) else t)(jnp.asarray(a)))
    B, Sq, D = 16, 96, 576
    Hq, Hkv, Sk, Dh = 32, 16, 512, 128
    assert Hq % Hkv == 0, (Hq, Hkv)
    return {
        "x": _w((lambda *s: _rng.normal(s) * 0.2)(B, Sq, D)),
        "k_cache": _w((lambda *s: _rng.normal(s) * 3.2)(B, Hkv, Sk, Dh)),
        "v_cache": _w((lambda *s: _rng.normal(s) * 0.05)(B, Hkv, Sk, Dh)),
        "wq": _w((lambda *s: _rng.normal(s) * 0.2)(D, Hq * Dh) * (D ** -0.5)),
        "wo": _w((lambda *s: _rng.normal(s) * 0.05)(Hq * Dh, D) * ((Hq * Dh) ** -0.5)),
    }

def reference(x, k_cache, v_cache, wq, wo):
    B, Sq, D = x.shape
    Hq, Dh = 32, 128
    Hkv = k_cache.shape[1]
    rep = Hq // Hkv
    q = (lambda x, *d: x.transpose(*d))((x @ wq).reshape(B, Sq, Hq, Dh), 0, 2, 1, 3)
    k = jnp.repeat(k_cache, rep, axis=1)
    v = jnp.repeat(v_cache, rep, axis=1)
    scores = jnp.einsum("bhqd,bhkd->bhqk", q, k) * (Dh ** -0.5)
    p = _softmax(scores, axis=-1)
    o = jnp.einsum("bhqk,bhkd->bhqd", p, v)
    return (lambda x, *d: x.transpose(*d))(o, 0, 2, 1, 3).reshape(B, Sq, Hq * Dh) @ wo
```

```python
import functools
import math
import jax
import jax.numpy as jnp
from jax import lax
import jax.experimental.pallas as pl
import jax.experimental.pallas.tpu as pltpu

_NT = (((1,), (1,)), ((), ()))

CFG = dict(p1='i', nloop=3, lag=1, osplit=3)


def build(cfg):
    @jax.jit
    def fn(x, k_cache, v_cache, wq, wo):
        B, Sq, D = x.shape
        _, Hkv, Sk, Dh = k_cache.shape
        Hq = wq.shape[1] // Dh
        rep = Hq // Hkv
        GB = 4
        NG = B // GB
        R = GB * Sq
        SUBW = 512
        NSUB = Hq * Dh // SUBW
        hps = SUBW // Dh
        qscale = Dh ** -0.5 * math.log2(math.e)
        DM = (D // 128) * 128
        OS = cfg['osplit']
        RT = R // OS
        S_X, S_WQ, S_WO = 0, NG, NG + NSUB + 1
        S_K = S_WO + 1
        S_V = S_K + NG
        S_O = S_V + NG
        NSEM = S_O + NG * OS

        def kernel(x_hbm, k_hbm, v_hbm, wq_hbm, wot_hbm, out_hbm,
                   x_buf, wq_buf, wot_buf, k_buf, v_buf, q_scr, out_buf, sems):
            def x_cp(g):
                return pltpu.make_async_copy(x_hbm.at[pl.ds(g * R, R)], x_buf.at[g], sems.at[S_X + g])

            def wq_cp(s):
                return pltpu.make_async_copy(wq_hbm.at[:, pl.ds(s * SUBW, SUBW)], wq_buf.at[s], sems.at[S_WQ + s])

            def wq0_cp(half):
                hw = SUBW // 2
                return pltpu.make_async_copy(wq_hbm.at[:, pl.ds(half * hw, hw)], wq_buf.at[0, :, pl.ds(half * hw, hw)],
                                             sems.at[S_WQ + (NSUB if half else 0)])

            def wo_cp():
                return pltpu.make_async_copy(wot_hbm, wot_buf, sems.at[S_WO])

            def k_cp(g):
                return pltpu.make_async_copy(k_hbm.at[pl.ds(g * GB, GB)], k_buf.at[g], sems.at[S_K + g])

            def v_cp(g):
                return pltpu.make_async_copy(v_hbm.at[pl.ds(g * GB, GB)], v_buf.at[g], sems.at[S_V + g])

            def out_cp(g, t):
                return pltpu.make_async_copy(out_buf.at[g, pl.ds(t * RT, RT)], out_hbm.at[pl.ds(g * R + t * RT, RT)],
                                             sems.at[S_O + g * OS + t])

            x_cp(0).start()
            if cfg['p1'] == 'ii':
                wq0_cp(0).start()
                wq0_cp(1).start()
            else:
                wq_cp(0).start()
            for g in range(1, NG):
                x_cp(g).start()
            for s in range(1, NSUB):
                wq_cp(s).start()
            k_cp(0).start()
            v_cp(0).start()
            wo_cp().start()
            for g in range(1, NG):
                k_cp(g).start()
                v_cp(g).start()

            def scoped(name, f):
                if not cfg.get('scopes'):
                    return f
                def w(*a):
                    with jax.named_scope(name):
                        return f(*a)
                return w

            def qproj(g, s, c0=0, c1=SUBW):
                q = jnp.dot(x_buf[g], wq_buf[s, :, c0:c1], preferred_element_type=jnp.float32)
                q = (q * qscale).astype(jnp.bfloat16)
                for hh in range(c0 // Dh, c1 // Dh):
                    q_scr[g, s * hps + hh] = q[:, hh * Dh - c0:(hh + 1) * Dh - c0]

            def peel():
                if cfg['p1'] == 'i':
                    x_cp(0).wait(); wq_cp(0).wait()
                    qproj(0, 0)
                    x_cp(1).wait(); x_cp(2).wait()
                    qproj(1, 0); qproj(2, 0)
                    x_cp(3).wait(); wq_cp(1).wait()
                    qproj(3, 0)
                    for g in range(NG):
                        qproj(g, 1)
                elif cfg['p1'] == 'ii':
                    x_cp(0).wait(); wq0_cp(0).wait()
                    qproj(0, 0, 0, SUBW // 2)
                    wq0_cp(1).wait()
                    qproj(0, 0, SUBW // 2, SUBW)
                    x_cp(1).wait()
                    qproj(1, 0)
                    x_cp(2).wait(); x_cp(3).wait()
                    qproj(2, 0); qproj(3, 0)
                    wq_cp(1).wait()
                    for g in range(NG):
                        qproj(g, 1)
                for s in range(2, NSUB):
                    wq_cp(s).wait()

            scoped('peel', peel)()
            nloop = cfg['nloop']
            spi = (NSUB - 2) // nloop

            def phase1(j, carry):
                for ss in range(spi):
                    for g in range(NG):
                        qproj(g, 2 + j * spi + ss)
                return carry

            if nloop == 1:
                scoped('p1', phase1)(0, 0)
            else:
                lax.fori_loop(0, nloop, scoped('p1', phase1), 0)
            wo_cp().wait()

            def phase2(g, carry):
                k_cp(g).wait()
                v_cp(g).wait()
                pairs = [(h, b) for h in range(Hkv) for b in range(GB)]
                o_ref = q_scr.at[NG]

                def qk(h, b):
                    q2 = jnp.concatenate(
                        [q_scr[g, h * rep + r, b * Sq:(b + 1) * Sq, :] for r in range(rep)], axis=0)
                    return lax.dot_general(q2, k_buf[g, b, h], _NT, preferred_element_type=jnp.float32)

                def pv(h, b, s):
                    m = jnp.max(s, axis=-1, keepdims=True)
                    p = jnp.exp2(s - m)
                    l = jnp.sum(p, axis=-1, keepdims=True)
                    o = jnp.dot(p.astype(jnp.bfloat16), v_buf[g, b, h], preferred_element_type=jnp.float32)
                    return o, l

                def fin(h, b, o, l):
                    r_ = pl.reciprocal(l, approx=False, full_range=False)
                    o = (o * r_).astype(jnp.bfloat16)
                    for r in range(rep):
                        o_ref[h * rep + r, b * Sq:(b + 1) * Sq, :] = o[r * Sq:(r + 1) * Sq]

                lag = cfg['lag']
                pend = []
                s_next = qk(*pairs[0])
                for i, (h, b) in enumerate(pairs):
                    s_cur = s_next
                    if i + 1 < len(pairs):
                        s_next = qk(*pairs[i + 1])
                    pend.append((h, b) + pv(h, b, s_cur))
                    if len(pend) > lag:
                        fin(*pend.pop(0))
                for t in pend:
                    fin(*t)

                o_all = jnp.concatenate([o_ref[h] for h in range(Hq)], axis=1)
                tail_t = lax.dot_general(wot_buf[DM:D, :], o_all, _NT, preferred_element_type=jnp.float32)
                tail_t = jnp.concatenate([tail_t, jnp.zeros((128 - (D - DM), R), jnp.float32)], axis=0)
                tail = tail_t.T
                out_buf[g, :, DM:D] = tail[:, :D - DM].astype(out_buf.dtype)
                for t in range(OS):
                    o_t = jnp.concatenate([o_ref[h, t * RT:(t + 1) * RT, :] for h in range(Hq)], axis=1)
                    res = lax.dot_general(o_t, wot_buf[0:DM, :], _NT, preferred_element_type=jnp.float32)
                    out_buf[g, t * RT:(t + 1) * RT, 0:DM] = res.astype(out_buf.dtype)
                    out_cp(g, t).start()
                return carry

            lax.fori_loop(0, NG, scoped('p2', phase2), 0)
            for g in range(NG):
                for t in range(OS):
                    out_cp(g, t).wait()

        hbm = pl.BlockSpec(memory_space=pltpu.HBM)
        bf = jnp.bfloat16
        out = pl.pallas_call(
            kernel,
            in_specs=[hbm] * 5,
            out_specs=hbm,
            out_shape=jax.ShapeDtypeStruct((B * Sq, D), x.dtype),
            scratch_shapes=[
                pltpu.VMEM((NG, R, D), bf),
                pltpu.VMEM((NSUB, D, SUBW), bf),
                pltpu.VMEM((D, Hq * Dh), bf),
                pltpu.VMEM((NG, GB, Hkv, Sk, Dh), bf),
                pltpu.VMEM((NG, GB, Hkv, Sk, Dh), bf),
                pltpu.VMEM((NG + 1, Hq, R, Dh), bf),
                pltpu.VMEM((NG, R, D), bf),
                pltpu.SemaphoreType.DMA((NSEM,)),
            ],
            compiler_params=pltpu.CompilerParams(vmem_limit_bytes=120 * 1024 * 1024),
        )(x.reshape(B * Sq, D), k_cache, v_cache, wq, wo.T)
        return out.reshape(B, Sq, D)
    return fn


pallas_standalone__gqa_block_cached__near_ridge_kernel = build(CFG)
```

```python
import math

import jax
import jax.numpy as jnp
from jax import lax
import jax.experimental.pallas as pl
import jax.experimental.pallas.tpu as pltpu

_NT = (((1,), (1,)), ((), ()))
_LANE = 128
_GB = 4
_WQ_CHUNK = 512
_N_LOOP = 3

_X_CUTS = (0, 192, 448, 1152, 1536)
_FIRST_DMAS = ("x0", "a", "b", "x1", "w1", "x2", "x3")
_STAGES = (
    (("x0", "a"), ((0, 96, 0, 0, 256), (96, 192, 0, 0, 256))),
    (("b",), ((0, 96, 0, 256, 512), (96, 192, 0, 256, 512))),
    (("x1",), ((192, 384, 0, 0, 512), (384, 448, 0, 0, 512))),
    (("w1",), ((0, 384, 1, 0, 512), (384, 448, 1, 0, 512))),
    (("x2",), ((448, 768, 0, 0, 512), (768, 1152, 0, 0, 512), (448, 768, 1, 0, 512))),
)
_OUT_PIECES = ((0, 128, 0, 576), (128, 128, 0, 576), (256, 128, 0, 384), (256, 128, 384, 192))


def _select(j, vals):
    if all(v == vals[0] for v in vals):
        return vals[0]
    step = vals[1] - vals[0]
    if all(v == vals[0] + i * step for i, v in enumerate(vals)):
        return vals[0] + j * step
    out = jnp.int32(vals[-1])
    for i in range(len(vals) - 2, -1, -1):
        out = jnp.where(j == i, jnp.int32(vals[i]), out)
    return out


@jax.jit
def pallas_standalone__gqa_block_cached__near_ridge_kernel(
    x: jax.Array,
    k_cache: jax.Array,
    v_cache: jax.Array,
    wq: jax.Array,
    wo: jax.Array,
):
    B, Sq, D = x.shape
    _, Hkv, Sk, Dh = k_cache.shape
    Hq = wq.shape[1] // Dh
    rep = Hq // Hkv
    assert (B, Sq, D, Hq, Hkv, Dh) == (16, 96, 576, 32, 16, 128), "schedule is tuned for these shapes"

    NG = B // _GB
    R = _GB * Sq
    M = B * Sq
    n_chunks = Hq * Dh // _WQ_CHUNK
    heads_per_chunk = _WQ_CHUNK // Dh
    half = _WQ_CHUNK // 2
    DM = (D // _LANE) * _LANE
    n_x = len(_X_CUTS) - 1
    n_out = len(_OUT_PIECES)
    q_scale = Dh ** -0.5 * math.log2(math.e)
    bf16, f32 = jnp.bfloat16, jnp.float32

    sem_x = 0
    sem_wq = sem_x + n_x
    sem_b = sem_wq + n_chunks
    sem_wo = sem_b + 1
    sem_k = sem_wo + 1
    sem_v = sem_k + NG
    sem_out = sem_v + NG
    n_sems = sem_out + NG * n_out

    done = {}
    for _, dots in _STAGES:
        for r0, r1, s, c0, c1 in dots:
            assert r0 // R == (r1 - 1) // R
            done[(r0 // R, s)] = done.get((r0 // R, s), 0) + (r1 - r0) * (c1 - c0)
    assert all(v == R * _WQ_CHUNK for v in done.values())
    rest = sorted(((g, s) for s in range(n_chunks) for g in range(NG) if (g, s) not in done),
                  key=lambda t: (max(t[1], 1), t[0], t[1]))
    per_iter = len(rest) // _N_LOOP
    assert per_iter * _N_LOOP == len(rest)

    def body(x_hbm, k_hbm, v_hbm, wq_hbm, wot_hbm, out_hbm,
             x_buf, wq_buf, wot_buf, k_buf, v_buf, qo_scr, out_buf, sems):
        def in_copy(name):
            if name in ("a", "b"):
                cols = pl.ds(0 if name == "a" else half, half)
                return pltpu.make_async_copy(wq_hbm.at[:, cols], wq_buf.at[0, :, cols],
                                             sems.at[sem_wq if name == "a" else sem_b])
            i = int(name[1:])
            if name[0] == "x":
                rows = pl.ds(_X_CUTS[i], _X_CUTS[i + 1] - _X_CUTS[i])
                return pltpu.make_async_copy(x_hbm.at[rows], x_buf.at[rows], sems.at[sem_x + i])
            return pltpu.make_async_copy(wq_hbm.at[:, pl.ds(i * _WQ_CHUNK, _WQ_CHUNK)],
                                         wq_buf.at[i], sems.at[sem_wq + i])

        def wo_copy():
            return pltpu.make_async_copy(wot_hbm, wot_buf, sems.at[sem_wo])

        def k_copy(g):
            return pltpu.make_async_copy(k_hbm.at[pl.ds(g * _GB, _GB)], k_buf.at[g], sems.at[sem_k + g])

        def v_copy(g):
            return pltpu.make_async_copy(v_hbm.at[pl.ds(g * _GB, _GB)], v_buf.at[g], sems.at[sem_v + g])

        def out_copy(g, t):
            r0, nr, c0, nc = _OUT_PIECES[t]
            sem = sems.at[sem_out + g * n_out + t]
            if nc == D:
                return pltpu.make_async_copy(out_buf.at[g, pl.ds(r0, nr)],
                                             out_hbm.at[pl.ds(g * R + r0, nr)], sem)
            return pltpu.make_async_copy(out_buf.at[g, pl.ds(r0, nr), pl.ds(c0, nc)],
                                         out_hbm.at[pl.ds(g * R + r0, nr), pl.ds(c0, nc)], sem)

        for name in _FIRST_DMAS + tuple("w%d" % s for s in range(2, n_chunks)):
            in_copy(name).start()
        k_copy(0).start()
        v_copy(0).start()
        wo_copy().start()
        for g in range(1, NG):
            k_copy(g).start()
            v_copy(g).start()

        def q_proj(xs, g, rows, s, c0, c1):
            q = jnp.dot(xs, wq_buf[s, :, c0:c1], preferred_element_type=f32)
            q = (q * q_scale).astype(bf16)
            for hh in range(c0 // Dh, c1 // Dh):
                qo_scr[g, s * heads_per_chunk + hh, rows, :] = q[:, hh * Dh - c0:(hh + 1) * Dh - c0]

        waited = {"w0"}
        for waits, dots in _STAGES:
            for name in waits:
                in_copy(name).wait()
                waited.add(name)
            for r0, r1, s, c0, c1 in dots:
                g = r0 // R
                q_proj(x_buf[r0:r1, :], g, slice(r0 - g * R, r1 - g * R), s, c0, c1)

        def missing(units):
            names = []
            for g, s in units:
                xs = ["x%d" % i for i in range(n_x) if _X_CUTS[i] < (g + 1) * R and _X_CUTS[i + 1] > g * R]
                for name in ["w%d" % s] + xs:
                    if name not in waited:
                        waited.add(name)
                        names.append(name)
            return names

        for name in missing(rest[:per_iter]):
            in_copy(name).wait()
        late = missing(rest[per_iter:])

        def phase1(j, carry):
            @pl.when(j == 1)
            def _():
                for name in late:
                    in_copy(name).wait()

            for i in range(per_iter):
                units = [rest[jj * per_iter + i] for jj in range(_N_LOOP)]
                g = _select(j, [u[0] for u in units])
                s = _select(j, [u[1] for u in units])
                xs = x_buf[pl.ds(pl.multiple_of(g * R, R), R), :]
                q_proj(xs, g, slice(0, R), s, 0, _WQ_CHUNK)
            return carry

        lax.fori_loop(0, _N_LOOP, phase1, 0)
        wo_copy().wait()

        o_ref = qo_scr.at[NG]
        pairs = [(h, b) for h in range(Hkv) for b in range(_GB)]

        def phase2(g, carry):
            k_copy(g).wait()
            v_copy(g).wait()

            def scores(h, b):
                q2 = jnp.concatenate(
                    [qo_scr[g, h * rep + r, b * Sq:(b + 1) * Sq, :] for r in range(rep)], axis=0)
                return lax.dot_general(q2, k_buf[g, b, h], _NT, preferred_element_type=f32)

            def weighted_values(h, b, s):
                p = jnp.exp2(s - jnp.max(s, axis=-1, keepdims=True))
                l = jnp.sum(p, axis=-1, keepdims=True)
                o = jnp.dot(p.astype(bf16), v_buf[g, b, h], preferred_element_type=f32)
                return o, l

            def normalise(h, b, o, l):
                o = (o * pl.reciprocal(l, approx=False, full_range=False)).astype(bf16)
                for r in range(rep):
                    o_ref[h * rep + r, b * Sq:(b + 1) * Sq, :] = o[r * Sq:(r + 1) * Sq]

            s_next = scores(*pairs[0])
            pending = None
            for i, (h, b) in enumerate(pairs):
                s_cur = s_next
                if i + 1 < len(pairs):
                    s_next = scores(*pairs[i + 1])
                cur = (h, b) + weighted_values(h, b, s_cur)
                if pending is not None:
                    normalise(*pending)
                pending = cur
            normalise(*pending)

            def o_rows(r0, nr):
                return jnp.concatenate([o_ref[h, r0:r0 + nr, :] for h in range(Hq)], axis=1)

            tail_t = lax.dot_general(wot_buf[DM:D, :], o_rows(0, R), _NT, preferred_element_type=f32)
            tail_t = jnp.concatenate([tail_t, jnp.zeros((_LANE - (D - DM), R), f32)], axis=0)
            out_buf[g, :, DM:D] = tail_t.T[:, :D - DM].astype(out_buf.dtype)
            for t, (r0, nr, c0, nc) in enumerate(_OUT_PIECES):
                c1 = min(c0 + nc, DM)
                res = lax.dot_general(o_rows(r0, nr), wot_buf[c0:c1, :], _NT, preferred_element_type=f32)
                out_buf[g, r0:r0 + nr, c0:c1] = res.astype(out_buf.dtype)
                out_copy(g, t).start()
            return carry

        lax.fori_loop(0, NG, phase2, 0)
        for g in range(NG):
            for t in range(n_out):
                out_copy(g, t).wait()

    def kernel(*refs):
        def once(_, carry):
            body(*refs)
            return carry

        lax.fori_loop(0, pl.program_id(0) + 1, once, 0)

    hbm = pl.BlockSpec(memory_space=pltpu.HBM)
    out = pl.pallas_call(
        kernel,
        grid=(1,),
        in_specs=[hbm] * 5,
        out_specs=hbm,
        out_shape=jax.ShapeDtypeStruct((M, D), x.dtype),
        scratch_shapes=[
            pltpu.VMEM((M, D), bf16),
            pltpu.VMEM((n_chunks, D, _WQ_CHUNK), bf16),
            pltpu.VMEM((D, Hq * Dh), bf16),
            pltpu.VMEM((NG, _GB, Hkv, Sk, Dh), bf16),
            pltpu.VMEM((NG, _GB, Hkv, Sk, Dh), bf16),
            pltpu.VMEM((NG + 1, Hq, R, Dh), bf16),
            pltpu.VMEM((NG, R, D), bf16),
            pltpu.SemaphoreType.DMA((n_sems,)),
        ],
        compiler_params=pltpu.CompilerParams(
            dimension_semantics=("arbitrary",),
            vmem_limit_bytes=120 * 1024 * 1024,
            disable_semaphore_checks=True,
        ),
    )(x.reshape(M, D), k_cache, v_cache, wq, wo.T)
    return out.reshape(B, Sq, D)
```

```python
import math

import jax
import jax.numpy as jnp
from jax import lax
import jax.experimental.pallas as pl
import jax.experimental.pallas.tpu as pltpu

_NT = (((1,), (1,)), ((), ()))
_LANE = 128
_GB = 4
_WQ_CHUNK = 512
_N_LOOP = 3
_VB = 16

_X_CUTS = (0, 192, 448, 1152, 1536)
_FIRST_DMAS = ("x0", "a", "b", "x1", "w1", "xv", "x2", "x3")
_STAGES = (
    (("x0", "a"), ((0, 96, 0, 0, 256), (96, 192, 0, 0, 256))),
    (("b",), ((0, 96, 0, 256, 512), (96, 192, 0, 256, 512))),
    (("x1",), ((192, 384, 0, 0, 512), (384, 448, 0, 0, 512))),
    (("w1",), ((0, 384, 1, 0, 512), (384, 448, 1, 0, 512))),
    (("xv", "x2"), ((448, 768, 0, 0, 512), (768, 1152, 0, 0, 512), (448, 768, 1, 0, 512))),
)
_OUT_PIECES = ((0, 128, 0, 576), (128, 128, 0, 576), (256, 128, 0, 384), (256, 128, 384, 192))


def _select(j, vals):
    if all(v == vals[0] for v in vals):
        return vals[0]
    step = vals[1] - vals[0]
    if all(v == vals[0] + i * step for i, v in enumerate(vals)):
        return vals[0] + j * step
    out = jnp.int32(vals[-1])
    for i in range(len(vals) - 2, -1, -1):
        out = jnp.where(j == i, jnp.int32(vals[i]), out)
    return out


@jax.jit
def pallas_standalone__gqa_block_cached__near_ridge_kernel(
    x: jax.Array,
    k_cache: jax.Array,
    v_cache: jax.Array,
    wq: jax.Array,
    wo: jax.Array,
):
    B, Sq, D = x.shape
    _, Hkv, Sk, Dh = k_cache.shape
    Hq = wq.shape[1] // Dh
    rep = Hq // Hkv
    assert (B, Sq, D, Hq, Hkv, Dh) == (16, 96, 576, 32, 16, 128), "schedule is tuned for these shapes"

    NG = B // _GB
    R = _GB * Sq
    M = B * Sq
    n_chunks = Hq * Dh // _WQ_CHUNK
    heads_per_chunk = _WQ_CHUNK // Dh
    half = _WQ_CHUNK // 2
    DM = (D // _LANE) * _LANE
    DT = D - DM
    blocks = R // _LANE
    n_x = len(_X_CUTS) - 1
    n_out = len(_OUT_PIECES)
    q_scale = Dh ** -0.5 * math.log2(math.e)
    bf16, f32 = jnp.bfloat16, jnp.float32

    sem_x = 0
    sem_wq = sem_x + n_x
    sem_b = sem_wq + n_chunks
    sem_xv = sem_b + 1
    sem_wo = sem_xv + 1
    sem_k = sem_wo + 1
    sem_v = sem_k + NG
    sem_out = sem_v + NG
    n_sems = sem_out + NG * n_out

    done = {}
    for _, dots in _STAGES:
        for r0, r1, s, c0, c1 in dots:
            assert r0 // R == (r1 - 1) // R
            done[(r0 // R, s)] = done.get((r0 // R, s), 0) + (r1 - r0) * (c1 - c0)
    assert all(v == R * _WQ_CHUNK for v in done.values())
    rest = sorted(((g, s) for s in range(n_chunks) for g in range(NG) if (g, s) not in done),
                  key=lambda t: (max(t[1], 1), t[0], t[1]))
    per_iter = len(rest) // _N_LOOP
    assert per_iter * _N_LOOP == len(rest)

    def body(x_hbm, x3_hbm, k_hbm, v_hbm, wq_hbm, wot_hbm, out_hbm,
             x_buf, wq_buf, wot_buf, k_buf, v_buf, qo_scr, out_buf, xv_buf, xb_scr, sems):
        def in_copy(name):
            if name in ("a", "b"):
                cols = pl.ds(0 if name == "a" else half, half)
                return pltpu.make_async_copy(wq_hbm.at[:, cols], wq_buf.at[0, :, cols],
                                             sems.at[sem_wq if name == "a" else sem_b])
            if name == "xv":
                return pltpu.make_async_copy(x3_hbm.at[:, pl.ds(_LANE - _VB, _VB), pl.ds(DM, DT)], xv_buf, sems.at[sem_xv])
            i = int(name[1:])
            if name[0] == "x":
                rows = pl.ds(_X_CUTS[i], _X_CUTS[i + 1] - _X_CUTS[i])
                return pltpu.make_async_copy(x_hbm.at[rows], x_buf.at[rows], sems.at[sem_x + i])
            return pltpu.make_async_copy(wq_hbm.at[:, pl.ds(i * _WQ_CHUNK, _WQ_CHUNK)],
                                         wq_buf.at[i], sems.at[sem_wq + i])

        def wo_copy():
            return pltpu.make_async_copy(wot_hbm, wot_buf, sems.at[sem_wo])

        def k_copy(g):
            return pltpu.make_async_copy(k_hbm.at[pl.ds(g * _GB, _GB)], k_buf.at[g], sems.at[sem_k + g])

        def v_copy(g):
            return pltpu.make_async_copy(v_hbm.at[pl.ds(g * _GB, _GB)], v_buf.at[g], sems.at[sem_v + g])

        def out_copy(g, t):
            r0, nr, c0, nc = _OUT_PIECES[t]
            sem = sems.at[sem_out + g * n_out + t]
            if nc == D:
                return pltpu.make_async_copy(out_buf.at[g, pl.ds(r0, nr)],
                                             out_hbm.at[pl.ds(g * R + r0, nr)], sem)
            return pltpu.make_async_copy(out_buf.at[g, pl.ds(r0, nr), pl.ds(c0, nc)],
                                         out_hbm.at[pl.ds(g * R + r0, nr), pl.ds(c0, nc)], sem)

        for name in _FIRST_DMAS + tuple("w%d" % s for s in range(2, n_chunks)):
            in_copy(name).start()
        k_copy(0).start()
        v_copy(0).start()
        wo_copy().start()
        for g in range(1, NG):
            k_copy(g).start()
            v_copy(g).start()

        def store_q(q, g, rows, s, c0, c1):
            q = (q * q_scale).astype(bf16)
            for hh in range(c0 // Dh, c1 // Dh):
                qo_scr[g, s * heads_per_chunk + hh, rows, :] = q[:, hh * Dh - c0:(hh + 1) * Dh - c0]

        waited = {"w0"}
        for waits, dots in _STAGES:
            for name in waits:
                in_copy(name).wait()
                waited.add(name)
            if "xv" in waits:
                for blk in range(NG * blocks):
                    xt = xv_buf[blk].astype(f32)
                    for k in range(DT):
                        xb_scr[blk, k] = jnp.broadcast_to(xt[:, k:k + 1], (_VB, _LANE))
            for r0, r1, s, c0, c1 in dots:
                g = r0 // R
                q = jnp.dot(x_buf[r0:r1, :], wq_buf[s, :, c0:c1], preferred_element_type=f32)
                store_q(q, g, slice(r0 - g * R, r1 - g * R), s, c0, c1)


        def q_unit(g, s):
            base = pl.multiple_of(g * R, _LANE)
            keep = _LANE - _VB
            main = jnp.dot(x_buf[pl.ds(base, R), 0:DM], wq_buf[s, 0:DM, :], preferred_element_type=f32)
            x_tail = jnp.concatenate(
                [x_buf[pl.ds(base + e * _LANE, keep), DM:D] for e in range(blocks)], axis=0)
            tail = jnp.dot(x_tail, wq_buf[s, DM:D, :], preferred_element_type=f32)

            tiles = _WQ_CHUNK // _LANE
            acc = [[None] * tiles for _ in range(blocks * _VB // 8)]
            for k in range(DT):
                w = [jnp.broadcast_to(wq_buf[s, DM + k:DM + k + 1, c * _LANE:(c + 1) * _LANE].astype(f32), (8, _LANE))
                     for c in range(tiles)]
                for rb in range(len(acc)):
                    e, o = divmod(rb * 8, _VB)
                    xv = xb_scr[g * blocks + e, k, o:o + 8, :]
                    for c in range(tiles):
                        t = xv * w[c]
                        acc[rb][c] = t if acc[rb][c] is None else acc[rb][c] + t
            vpu = jnp.concatenate([jnp.concatenate(a, axis=1) for a in acc], axis=0)

            parts = []
            for e in range(blocks):
                parts += [tail[e * keep:(e + 1) * keep], vpu[e * _VB:(e + 1) * _VB]]
            store_q(main + jnp.concatenate(parts, axis=0), g, slice(0, R), s, 0, _WQ_CHUNK)

        def missing(units):
            names = []
            for g, s in units:
                xs = ["x%d" % i for i in range(n_x) if _X_CUTS[i] < (g + 1) * R and _X_CUTS[i + 1] > g * R]
                for name in ["w%d" % s] + xs:
                    if name not in waited:
                        waited.add(name)
                        names.append(name)
            return names

        for name in missing(rest[:per_iter]):
            in_copy(name).wait()
        late = missing(rest[per_iter:])

        def phase1(j, carry):
            @pl.when(j == 1)
            def _():
                for name in late:
                    in_copy(name).wait()

            for i in range(per_iter):
                units = [rest[jj * per_iter + i] for jj in range(_N_LOOP)]
                q_unit(_select(j, [u[0] for u in units]), _select(j, [u[1] for u in units]))
            return carry

        lax.fori_loop(0, _N_LOOP, phase1, 0)
        wo_copy().wait()

        o_ref = qo_scr.at[NG]
        pairs = [(h, b) for h in range(Hkv) for b in range(_GB)]

        def phase2(g, carry):
            k_copy(g).wait()
            v_copy(g).wait()

            def scores(h, b):
                q2 = jnp.concatenate(
                    [qo_scr[g, h * rep + r, b * Sq:(b + 1) * Sq, :] for r in range(rep)], axis=0)
                return lax.dot_general(q2, k_buf[g, b, h], _NT, preferred_element_type=f32)

            def weighted_values(h, b, s):
                p = jnp.exp2(s - jnp.max(s, axis=-1, keepdims=True))
                l = jnp.sum(p, axis=-1, keepdims=True)
                o = jnp.dot(p.astype(bf16), v_buf[g, b, h], preferred_element_type=f32)
                return o, l

            def normalise(h, b, o, l):
                o = (o * pl.reciprocal(l, approx=False, full_range=False)).astype(bf16)
                for r in range(rep):
                    o_ref[h * rep + r, b * Sq:(b + 1) * Sq, :] = o[r * Sq:(r + 1) * Sq]

            s_next = scores(*pairs[0])
            pending = None
            for i, (h, b) in enumerate(pairs):
                s_cur = s_next
                if i + 1 < len(pairs):
                    s_next = scores(*pairs[i + 1])
                cur = (h, b) + weighted_values(h, b, s_cur)
                if pending is not None:
                    normalise(*pending)
                pending = cur
            normalise(*pending)

            def o_rows(r0, nr):
                return jnp.concatenate([o_ref[h, r0:r0 + nr, :] for h in range(Hq)], axis=1)

            tail_t = lax.dot_general(wot_buf[DM:D, :], o_rows(0, R), _NT, preferred_element_type=f32)
            tail_t = jnp.concatenate([tail_t, jnp.zeros((_LANE - (D - DM), R), f32)], axis=0)
            out_buf[g, :, DM:D] = tail_t.T[:, :D - DM].astype(out_buf.dtype)
            for t, (r0, nr, c0, nc) in enumerate(_OUT_PIECES):
                c1 = min(c0 + nc, DM)
                res = lax.dot_general(o_rows(r0, nr), wot_buf[c0:c1, :], _NT, preferred_element_type=f32)
                out_buf[g, r0:r0 + nr, c0:c1] = res.astype(out_buf.dtype)
                out_copy(g, t).start()
            return carry

        lax.fori_loop(0, NG, phase2, 0)
        for g in range(NG):
            for t in range(n_out):
                out_copy(g, t).wait()

    def kernel(*refs):
        def once(_, carry):
            body(*refs)
            return carry

        lax.fori_loop(0, pl.program_id(0) + 1, once, 0)

    hbm = pl.BlockSpec(memory_space=pltpu.HBM)
    out = pl.pallas_call(
        kernel,
        grid=(1,),
        in_specs=[hbm] * 6,
        out_specs=hbm,
        out_shape=jax.ShapeDtypeStruct((M, D), x.dtype),
        scratch_shapes=[
            pltpu.VMEM((M, D), bf16),
            pltpu.VMEM((n_chunks, D, _WQ_CHUNK), bf16),
            pltpu.VMEM((D, Hq * Dh), bf16),
            pltpu.VMEM((NG, _GB, Hkv, Sk, Dh), bf16),
            pltpu.VMEM((NG, _GB, Hkv, Sk, Dh), bf16),
            pltpu.VMEM((NG + 1, Hq, R, Dh), bf16),
            pltpu.VMEM((NG, R, D), bf16),
            pltpu.VMEM((NG * blocks, _VB, DT), bf16),
            pltpu.VMEM((NG * blocks, DT, _VB, _LANE), f32),
            pltpu.SemaphoreType.DMA((n_sems,)),
        ],
        compiler_params=pltpu.CompilerParams(
            dimension_semantics=("arbitrary",),
            vmem_limit_bytes=120 * 1024 * 1024,
            disable_semaphore_checks=True,
        ),
    )(x.reshape(M, D), x.reshape(M // _LANE, _LANE, D), k_cache, v_cache, wq, wo.T)
    return out.reshape(B, Sq, D)
```

```python
import math

import jax
import jax.numpy as jnp
from jax import lax
import jax.experimental.pallas as pl
import jax.experimental.pallas.tpu as pltpu

_NT = (((1,), (1,)), ((), ()))
_LANE = 128
_GB = 4
_WQ_CHUNK = 512
_N_LOOP = 3
_VB = 16
_NOW = (128, 112)
_LATE = (192, 96)
_GROUP0_SLOTS = (0, 5)
_LATE_HEAD_START = 2

_X_CUTS = (0, 192, 448, 1152, 1536)
_FIRST_DMAS = ("x0", "a", "b", "x1", "w1", "now", "late", "x2", "x3")
_STAGES = (
    (("x0", "a"), ((0, 96, 0, 0, 256), (96, 192, 0, 0, 256))),
    (("b",), ((0, 96, 0, 256, 512), (96, 192, 0, 256, 512))),
    (("x1",), ((192, 384, 0, 0, 512), (384, 448, 0, 0, 512))),
    (("w1",), ((0, 384, 1, 0, 512), (384, 448, 1, 0, 512))),
    (("now", "late", "x2"), ((448, 768, 0, 0, 512), (768, 1152, 0, 0, 512), (448, 768, 1, 0, 512))),
)
_OUT_PIECES = ((0, 128, 0, 576), (128, 128, 0, 576), (256, 128, 0, 384), (256, 128, 384, 192))


def _select(j, vals):
    if all(v == vals[0] for v in vals):
        return vals[0]
    step = vals[1] - vals[0]
    if all(v == vals[0] + i * step for i, v in enumerate(vals)):
        return vals[0] + j * step
    out = jnp.int32(vals[-1])
    for i in range(len(vals) - 2, -1, -1):
        out = jnp.where(j == i, jnp.int32(vals[i]), out)
    return out


@jax.jit
def pallas_standalone__gqa_block_cached__near_ridge_kernel(
    x: jax.Array,
    k_cache: jax.Array,
    v_cache: jax.Array,
    wq: jax.Array,
    wo: jax.Array,
):
    B, Sq, D = x.shape
    _, Hkv, Sk, Dh = k_cache.shape
    Hq = wq.shape[1] // Dh
    rep = Hq // Hkv
    assert (B, Sq, D, Hq, Hkv, Dh) == (16, 96, 576, 32, 16, 128), "schedule is tuned for these shapes"

    NG = B // _GB
    R = _GB * Sq
    M = B * Sq
    n_chunks = Hq * Dh // _WQ_CHUNK
    heads_per_chunk = _WQ_CHUNK // Dh
    half = _WQ_CHUNK // 2
    DM = (D // _LANE) * _LANE
    DT = D - DM
    now_rows = list(range(_NOW[1], R, _NOW[0]))
    late_rows = list(range(_LATE[1], R, _LATE[0]))
    n_now, n_late = len(now_rows), len(late_rows)
    n_x = len(_X_CUTS) - 1
    n_out = len(_OUT_PIECES)
    q_scale = Dh ** -0.5 * math.log2(math.e)
    bf16, f32 = jnp.bfloat16, jnp.float32

    sem_x = 0
    sem_wq = sem_x + n_x
    sem_b = sem_wq + n_chunks
    sem_now = sem_b + 1
    sem_late = sem_now + 1
    sem_wo = sem_late + 1
    sem_k = sem_wo + 1
    sem_v = sem_k + NG
    sem_out = sem_v + NG
    n_sems = sem_out + NG * n_out

    done = {}
    for _, dots in _STAGES:
        for r0, r1, s, c0, c1 in dots:
            assert r0 // R == (r1 - 1) // R
            done[(r0 // R, s)] = done.get((r0 // R, s), 0) + (r1 - r0) * (c1 - c0)
    assert all(v == R * _WQ_CHUNK for v in done.values())
    todo = sorted(((g, s) for s in range(n_chunks) for g in range(NG) if (g, s) not in done),
                  key=lambda t: (max(t[1], 1), t[0], t[1]))
    per_iter = len(todo) // _N_LOOP
    group0, others = [u for u in todo if u[0] == 0], [u for u in todo if u[0] != 0]
    assert per_iter * _N_LOOP == len(todo) and len(group0) == _N_LOOP * len(_GROUP0_SLOTS)
    units = [[(group0 if i in _GROUP0_SLOTS else others).pop(0) for i in range(per_iter)]
             for _ in range(_N_LOOP)]

    def body(x_hbm, x_now_hbm, x_late_hbm, k_hbm, v_hbm, wq_hbm, wot_hbm, out_hbm,
             x_buf, wq_buf, wot_buf, k_buf, v_buf, qo_scr, out_buf,
             x_now_buf, x_late_buf, xb_scr, q_main_scr, sems):
        def in_copy(name):
            if name in ("a", "b"):
                cols = pl.ds(0 if name == "a" else half, half)
                return pltpu.make_async_copy(wq_hbm.at[:, cols], wq_buf.at[0, :, cols],
                                             sems.at[sem_wq if name == "a" else sem_b])
            if name == "now":
                return pltpu.make_async_copy(x_now_hbm.at[:, pl.ds(_NOW[1], _VB), pl.ds(DM, DT)],
                                             x_now_buf, sems.at[sem_now])
            if name == "late":
                return pltpu.make_async_copy(x_late_hbm.at[:, pl.ds(_LATE[1], _VB), pl.ds(DM, DT)],
                                             x_late_buf, sems.at[sem_late])
            i = int(name[1:])
            if name[0] == "x":
                rows = pl.ds(_X_CUTS[i], _X_CUTS[i + 1] - _X_CUTS[i])
                return pltpu.make_async_copy(x_hbm.at[rows], x_buf.at[rows], sems.at[sem_x + i])
            return pltpu.make_async_copy(wq_hbm.at[:, pl.ds(i * _WQ_CHUNK, _WQ_CHUNK)],
                                         wq_buf.at[i], sems.at[sem_wq + i])

        def wo_copy():
            return pltpu.make_async_copy(wot_hbm, wot_buf, sems.at[sem_wo])

        def k_copy(g):
            return pltpu.make_async_copy(k_hbm.at[pl.ds(g * _GB, _GB)], k_buf.at[g], sems.at[sem_k + g])

        def v_copy(g):
            return pltpu.make_async_copy(v_hbm.at[pl.ds(g * _GB, _GB)], v_buf.at[g], sems.at[sem_v + g])

        def out_copy(g, t):
            r0, nr, c0, nc = _OUT_PIECES[t]
            sem = sems.at[sem_out + g * n_out + t]
            if nc == D:
                return pltpu.make_async_copy(out_buf.at[g, pl.ds(r0, nr)],
                                             out_hbm.at[pl.ds(g * R + r0, nr)], sem)
            return pltpu.make_async_copy(out_buf.at[g, pl.ds(r0, nr), pl.ds(c0, nc)],
                                         out_hbm.at[pl.ds(g * R + r0, nr), pl.ds(c0, nc)], sem)

        for name in _FIRST_DMAS + tuple("w%d" % s for s in range(2, n_chunks)):
            in_copy(name).start()
        k_copy(0).start()
        v_copy(0).start()
        wo_copy().start()
        for g in range(1, NG):
            k_copy(g).start()
            v_copy(g).start()

        def store_q(q, g, lo, hi, s, c0=0, c1=_WQ_CHUNK):
            q = (q * q_scale).astype(bf16)
            for hh in range(c0 // Dh, c1 // Dh):
                qo_scr[g, s * heads_per_chunk + hh, lo:hi, :] = q[:, hh * Dh - c0:(hh + 1) * Dh - c0]

        def q_unit(g, s, lo, hi, now, late):
            base = g * R if isinstance(g, int) else pl.multiple_of(g * R, _LANE)
            special = sorted(now + late)
            spans = [(a, b) for a, b in zip([lo] + [r + _VB for r in special], special + [hi]) if b > a]
            main = jnp.dot(x_buf[pl.ds(base + lo, hi - lo), 0:DM], wq_buf[s, 0:DM, :],
                           preferred_element_type=f32)
            x_tail = jnp.concatenate([x_buf[pl.ds(base + a, b - a), DM:D] for a, b in spans], axis=0)
            mxu_tail = jnp.dot(x_tail, wq_buf[s, DM:D, :], preferred_element_type=f32)
            vpu_tail = None
            for k in (range(DT) if now else ()):
                xk = jnp.tile(xb_scr[g, k, 0:n_now * _VB, :], (1, heads_per_chunk))
                t = xk * wq_buf[s, DM + k:DM + k + 1, :].astype(f32)
                vpu_tail = t if vpu_tail is None else vpu_tail + t

            run, run_lo, used = [], lo, 0
            for a, b in sorted(spans + [(r, r + _VB) for r in special]) + [(hi, hi)]:
                if a in now:
                    e = now_rows.index(a)
                    run.append(vpu_tail[e * _VB:(e + 1) * _VB])
                elif a in late or a == hi:
                    if run:
                        q = main[run_lo - lo:a - lo] + jnp.concatenate(run, axis=0)
                        store_q(q, g, run_lo, a, s)
                    run, run_lo = [], b
                    if a != hi:
                        e = late_rows.index(a)
                        for hh in range(heads_per_chunk):
                            q_main_scr[g, s * heads_per_chunk + hh, e * _VB:(e + 1) * _VB, :] = (
                                main[a - lo:b - lo, hh * Dh:(hh + 1) * Dh])
                else:
                    run.append(mxu_tail[used:used + b - a])
                    used += b - a

        waited = {"w0"}
        for waits, dots in _STAGES:
            for name in waits:
                in_copy(name).wait()
                waited.add(name)
            if "now" in waits:
                for g in range(NG):
                    blocks = [x_now_buf[g * n_now + e] for e in range(n_now)]
                    blocks += [x_late_buf[g * n_late + e] for e in range(n_late if g else 0)]
                    xt = jnp.concatenate(blocks, axis=0).astype(f32)
                    n = len(blocks) * _VB
                    for k in range(DT):
                        xb_scr[g, k, 0:n, :] = jnp.broadcast_to(xt[:, k:k + 1], (n, _LANE))
            for r0, r1, s, c0, c1 in dots:
                g = r0 // R
                lo, hi = r0 - g * R, r1 - g * R
                late = [r for r in late_rows if g and lo <= r < hi]
                if late:
                    assert (c0, c1) == (0, _WQ_CHUNK)
                    q_unit(g, s, lo, hi, [], late)
                else:
                    q = jnp.dot(x_buf[r0:r1, :], wq_buf[s, :, c0:c1], preferred_element_type=f32)
                    store_q(q, g, lo, hi, s, c0, c1)

        def missing(us):
            names = []
            for g, s in us:
                xs = ["x%d" % i for i in range(n_x) if _X_CUTS[i] < (g + 1) * R and _X_CUTS[i + 1] > g * R]
                for name in ["w%d" % s] + xs:
                    if name not in waited:
                        waited.add(name)
                        names.append(name)
            return names

        for name in missing(units[0]):
            in_copy(name).wait()
        remaining = missing(sum(units[1:], []))

        def phase1(j, carry):
            @pl.when(j == 1)
            def _():
                for name in remaining:
                    in_copy(name).wait()

            for i in range(per_iter):
                g = _select(j, [u[i][0] for u in units])
                s = _select(j, [u[i][1] for u in units])
                q_unit(g, s, 0, R, now_rows, [] if i in _GROUP0_SLOTS else late_rows)
            return carry

        lax.fori_loop(0, _N_LOOP, phase1, 0)
        wo_copy().wait()

        o_ref = qo_scr.at[NG]
        pairs = [(h, b) for h in range(Hkv) for b in range(_GB)]

        def phase2(g, carry):
            k_copy(g).wait()
            v_copy(g).wait()
            g_next = jnp.minimum(g + 1, NG - 1)

            def scores(h, b):
                q2 = jnp.concatenate(
                    [qo_scr[g, h * rep + r, b * Sq:(b + 1) * Sq, :] for r in range(rep)], axis=0)
                return lax.dot_general(q2, k_buf[g, b, h], _NT, preferred_element_type=f32)

            def weighted_values(h, b, s):
                p = jnp.exp2(s - jnp.max(s, axis=-1, keepdims=True))
                l = jnp.sum(p, axis=-1, keepdims=True)
                o = jnp.dot(p.astype(bf16), v_buf[g, b, h], preferred_element_type=f32)
                return o, l

            def normalise(h, b, o, l):
                o = (o * pl.reciprocal(l, approx=False, full_range=False)).astype(bf16)
                for r in range(rep):
                    o_ref[h * rep + r, b * Sq:(b + 1) * Sq, :] = o[r * Sq:(r + 1) * Sq]

            def finish_late(head, e):
                s, c = divmod(head, heads_per_chunk)
                acc = q_main_scr[g_next, head, e * _VB:(e + 1) * _VB, :]
                for k in range(DT):
                    w = wq_buf[s, DM + k:DM + k + 1, c * Dh:(c + 1) * Dh].astype(f32)
                    acc = acc + xb_scr[g_next, k, (n_now + e) * _VB:(n_now + e + 1) * _VB, :] * w
                qo_scr[g_next, head, late_rows[e]:late_rows[e] + _VB, :] = (acc * q_scale).astype(bf16)

            late_todo = [(head, e) for head in range(Hq) for e in range(n_late)]
            s_next = scores(*pairs[0])
            for _ in range(_LATE_HEAD_START):
                finish_late(*late_todo.pop(0))
            pending = None
            for i, (h, b) in enumerate(pairs):
                s_cur = s_next
                if i + 1 < len(pairs):
                    s_next = scores(*pairs[i + 1])
                cur = (h, b) + weighted_values(h, b, s_cur)
                if pending is not None:
                    normalise(*pending)
                if late_todo:
                    finish_late(*late_todo.pop(0))
                pending = cur
            normalise(*pending)
            assert not late_todo

            def o_rows(r0, nr):
                return jnp.concatenate([o_ref[h, r0:r0 + nr, :] for h in range(Hq)], axis=1)

            tail_t = lax.dot_general(wot_buf[DM:D, :], o_rows(0, R), _NT, preferred_element_type=f32)
            tail_t = jnp.concatenate([tail_t, jnp.zeros((_LANE - DT, R), f32)], axis=0)
            out_buf[g, :, DM:D] = tail_t.T[:, :DT].astype(out_buf.dtype)
            for t, (r0, nr, c0, nc) in enumerate(_OUT_PIECES):
                c1 = min(c0 + nc, DM)
                res = lax.dot_general(o_rows(r0, nr), wot_buf[c0:c1, :], _NT, preferred_element_type=f32)
                out_buf[g, r0:r0 + nr, c0:c1] = res.astype(out_buf.dtype)
                out_copy(g, t).start()
            return carry

        lax.fori_loop(0, NG, phase2, 0)
        for g in range(NG):
            for t in range(n_out):
                out_copy(g, t).wait()

    def kernel(*refs):
        def once(_, carry):
            body(*refs)
            return carry

        lax.fori_loop(0, pl.program_id(0) + 1, once, 0)

    hbm = pl.BlockSpec(memory_space=pltpu.HBM)
    out = pl.pallas_call(
        kernel,
        grid=(1,),
        in_specs=[hbm] * 7,
        out_specs=hbm,
        out_shape=jax.ShapeDtypeStruct((M, D), x.dtype),
        scratch_shapes=[
            pltpu.VMEM((M, D), bf16),
            pltpu.VMEM((n_chunks, D, _WQ_CHUNK), bf16),
            pltpu.VMEM((D, Hq * Dh), bf16),
            pltpu.VMEM((NG, _GB, Hkv, Sk, Dh), bf16),
            pltpu.VMEM((NG, _GB, Hkv, Sk, Dh), bf16),
            pltpu.VMEM((NG + 1, Hq, R, Dh), bf16),
            pltpu.VMEM((NG, R, D), bf16),
            pltpu.VMEM((NG * n_now, _VB, DT), bf16),
            pltpu.VMEM((NG * n_late, _VB, DT), bf16),
            pltpu.VMEM((NG, DT, (n_now + n_late) * _VB, _LANE), f32),
            pltpu.VMEM((NG, Hq, n_late * _VB, Dh), f32),
            pltpu.SemaphoreType.DMA((n_sems,)),
        ],
        compiler_params=pltpu.CompilerParams(
            dimension_semantics=("arbitrary",),
            vmem_limit_bytes=120 * 1024 * 1024,
            disable_semaphore_checks=True,
        ),
    )(x.reshape(M, D), x.reshape(M // _NOW[0], _NOW[0], D), x.reshape(M // _LATE[0], _LATE[0], D),
      k_cache, v_cache, wq, wo.T)
    return out.reshape(B, Sq, D)
```

```python
import math

import jax
import jax.numpy as jnp
from jax import lax
import jax.experimental.pallas as pl
import jax.experimental.pallas.tpu as pltpu

_NT = (((1,), (1,)), ((), ()))
_LANE = 128
_GB = 4
_WQ_CHUNK = 512
_N_LOOP = 3
_VB = 16
_NOW = (128, 112)
_LATE = (192, 96)
_GROUP0_SLOTS = (0, 5)
_LATE_HEAD_START = 2

_X_CUTS = (0, 192, 448, 1152, 1536)
_FIRST_DMAS = ("x0", "a", "b", "x1", "w1", "now", "late", "x2", "x3")
_STAGES = (
    (("x0", "a"), ((0, 96, 0, 0, 256), (96, 192, 0, 0, 256))),
    (("b",), ((0, 96, 0, 256, 512), (96, 192, 0, 256, 512))),
    (("x1",), ((192, 384, 0, 0, 512), (384, 448, 0, 0, 512))),
    (("w1",), ((0, 384, 1, 0, 512), (384, 448, 1, 0, 512))),
    (("now", "late", "x2"), ((448, 768, 0, 0, 512), (768, 1152, 0, 0, 512), (448, 768, 1, 0, 512))),
)
_OUT_PIECES = ((0, 128, 0, 576), (128, 128, 0, 576), (256, 128, 0, 384), (256, 128, 384, 192))


def _select(j, vals):
    if all(v == vals[0] for v in vals):
        return vals[0]
    step = vals[1] - vals[0]
    if all(v == vals[0] + i * step for i, v in enumerate(vals)):
        return vals[0] + j * step
    out = jnp.int32(vals[-1])
    for i in range(len(vals) - 2, -1, -1):
        out = jnp.where(j == i, jnp.int32(vals[i]), out)
    return out


@jax.jit
def pallas_standalone__gqa_block_cached__near_ridge_kernel(
    x: jax.Array,
    k_cache: jax.Array,
    v_cache: jax.Array,
    wq: jax.Array,
    wo: jax.Array,
):
    B, Sq, D = x.shape
    _, Hkv, Sk, Dh = k_cache.shape
    Hq = wq.shape[1] // Dh
    rep = Hq // Hkv
    assert (B, Sq, D, Hq, Hkv, Dh) == (16, 96, 576, 32, 16, 128), "schedule is tuned for these shapes"

    NG = B // _GB
    R = _GB * Sq
    M = B * Sq
    n_chunks = Hq * Dh // _WQ_CHUNK
    heads_per_chunk = _WQ_CHUNK // Dh
    half = _WQ_CHUNK // 2
    DM = (D // _LANE) * _LANE
    DT = D - DM
    now_rows = list(range(_NOW[1], R, _NOW[0]))
    late_rows = list(range(_LATE[1], R, _LATE[0]))
    n_now, n_late = len(now_rows), len(late_rows)
    n_x = len(_X_CUTS) - 1
    n_out = len(_OUT_PIECES)
    q_scale = Dh ** -0.5 * math.log2(math.e)
    bf16, f32 = jnp.bfloat16, jnp.float32

    sem_x = 0
    sem_wq = sem_x + n_x
    sem_b = sem_wq + n_chunks
    sem_now = sem_b + 1
    sem_late = sem_now + 1
    sem_wo = sem_late + 1
    sem_k = sem_wo + 1
    sem_v = sem_k + NG
    sem_out = sem_v + NG
    n_sems = sem_out + NG * n_out

    done = {}
    for _, dots in _STAGES:
        for r0, r1, s, c0, c1 in dots:
            assert r0 // R == (r1 - 1) // R
            done[(r0 // R, s)] = done.get((r0 // R, s), 0) + (r1 - r0) * (c1 - c0)
    assert all(v == R * _WQ_CHUNK for v in done.values())
    todo = sorted(((g, s) for s in range(n_chunks) for g in range(NG) if (g, s) not in done),
                  key=lambda t: (max(t[1], 1), t[0], t[1]))
    per_iter = len(todo) // _N_LOOP
    group0, others = [u for u in todo if u[0] == 0], [u for u in todo if u[0] != 0]
    assert per_iter * _N_LOOP == len(todo) and len(group0) == _N_LOOP * len(_GROUP0_SLOTS)
    units = [[(group0 if i in _GROUP0_SLOTS else others).pop(0) for i in range(per_iter)]
             for _ in range(_N_LOOP)]

    def body(x_hbm, x_now_hbm, x_late_hbm, k_hbm, v_hbm, wq_hbm, wot_hbm, out_hbm,
             x_buf, wq_buf, wot_buf, k_buf, v_buf, qo_scr, out_buf,
             x_now_buf, x_late_buf, xb_scr, q_main_scr, sems):
        def in_copy(name):
            if name in ("a", "b"):
                cols = pl.ds(0 if name == "a" else half, half)
                return pltpu.make_async_copy(wq_hbm.at[:, cols], wq_buf.at[0, :, cols],
                                             sems.at[sem_wq if name == "a" else sem_b])
            if name == "now":
                return pltpu.make_async_copy(x_now_hbm.at[:, pl.ds(_NOW[1], _VB), pl.ds(DM, DT)],
                                             x_now_buf, sems.at[sem_now])
            if name == "late":
                return pltpu.make_async_copy(x_late_hbm.at[:, pl.ds(_LATE[1], _VB), pl.ds(DM, DT)],
                                             x_late_buf, sems.at[sem_late])
            i = int(name[1:])
            if name[0] == "x":
                rows = pl.ds(_X_CUTS[i], _X_CUTS[i + 1] - _X_CUTS[i])
                return pltpu.make_async_copy(x_hbm.at[rows], x_buf.at[rows], sems.at[sem_x + i])
            return pltpu.make_async_copy(wq_hbm.at[:, pl.ds(i * _WQ_CHUNK, _WQ_CHUNK)],
                                         wq_buf.at[i], sems.at[sem_wq + i])

        def wo_copy():
            return pltpu.make_async_copy(wot_hbm, wot_buf, sems.at[sem_wo])

        def k_copy(g):
            return pltpu.make_async_copy(k_hbm.at[pl.ds(g * _GB, _GB)], k_buf.at[g], sems.at[sem_k + g])

        def v_copy(g):
            return pltpu.make_async_copy(v_hbm.at[pl.ds(g * _GB, _GB)], v_buf.at[g], sems.at[sem_v + g])

        def out_copy(g, t):
            r0, nr, c0, nc = _OUT_PIECES[t]
            sem = sems.at[sem_out + g * n_out + t]
            if nc == D:
                return pltpu.make_async_copy(out_buf.at[g, pl.ds(r0, nr)],
                                             out_hbm.at[pl.ds(g * R + r0, nr)], sem)
            return pltpu.make_async_copy(out_buf.at[g, pl.ds(r0, nr), pl.ds(c0, nc)],
                                         out_hbm.at[pl.ds(g * R + r0, nr), pl.ds(c0, nc)], sem)

        for name in _FIRST_DMAS + tuple("w%d" % s for s in range(2, n_chunks)):
            in_copy(name).start()
        k_copy(0).start()
        v_copy(0).start()
        wo_copy().start()
        for g in range(1, NG):
            k_copy(g).start()
            v_copy(g).start()

        def store_q(q, g, lo, hi, s, c0=0, c1=_WQ_CHUNK):
            q = (q * q_scale).astype(bf16)
            for hh in range(c0 // Dh, c1 // Dh):
                qo_scr[g, s * heads_per_chunk + hh, lo:hi, :] = q[:, hh * Dh - c0:(hh + 1) * Dh - c0]

        def q_unit(g, s, lo, hi, now, late):
            base = g * R if isinstance(g, int) else pl.multiple_of(g * R, _LANE)
            special = sorted(now + late)
            spans = [(a, b) for a, b in zip([lo] + [r + _VB for r in special], special + [hi]) if b > a]
            main = jnp.dot(x_buf[pl.ds(base + lo, hi - lo), 0:DM], wq_buf[s, 0:DM, :],
                           preferred_element_type=f32)
            x_tail = jnp.concatenate([x_buf[pl.ds(base + a, b - a), DM:D] for a, b in spans], axis=0)
            mxu_tail = jnp.dot(x_tail, wq_buf[s, DM:D, :], preferred_element_type=f32)
            if now:
                w = wq_buf[s, DM:D, :].astype(f32)
                xb = xb_scr[g, :, 0:n_now * _VB, :]
                vpu_tail = jnp.tile(xb[0], (1, heads_per_chunk)) * w[0:1]
                for k in range(1, DT):
                    vpu_tail = vpu_tail + jnp.tile(xb[k], (1, heads_per_chunk)) * w[k:k + 1]

            run, run_lo, used = [], lo, 0
            for a, b in sorted(spans + [(r, r + _VB) for r in special]) + [(hi, hi)]:
                if a in now:
                    e = now_rows.index(a)
                    run.append(vpu_tail[e * _VB:(e + 1) * _VB])
                elif a in late or a == hi:
                    if run:
                        q = main[run_lo - lo:a - lo] + jnp.concatenate(run, axis=0)
                        store_q(q, g, run_lo, a, s)
                    run, run_lo = [], b
                    if a != hi:
                        e = late_rows.index(a)
                        for hh in range(heads_per_chunk):
                            q_main_scr[g, s * heads_per_chunk + hh, e * _VB:(e + 1) * _VB, :] = (
                                main[a - lo:b - lo, hh * Dh:(hh + 1) * Dh])
                else:
                    run.append(mxu_tail[used:used + b - a])
                    used += b - a

        waited = {"w0"}
        for waits, dots in _STAGES:
            for name in waits:
                in_copy(name).wait()
                waited.add(name)
            if "now" in waits:
                for g in range(NG):
                    blocks = [x_now_buf[g * n_now + e] for e in range(n_now)]
                    blocks += [x_late_buf[g * n_late + e] for e in range(n_late if g else 0)]
                    xt = jnp.concatenate(blocks, axis=0).astype(f32)
                    n = len(blocks) * _VB
                    for k in range(DT):
                        xb_scr[g, k, 0:n, :] = jnp.broadcast_to(xt[:, k:k + 1], (n, _LANE))
            for r0, r1, s, c0, c1 in dots:
                g = r0 // R
                lo, hi = r0 - g * R, r1 - g * R
                late = [r for r in late_rows if g and lo <= r < hi]
                if late:
                    assert (c0, c1) == (0, _WQ_CHUNK)
                    q_unit(g, s, lo, hi, [], late)
                else:
                    q = jnp.dot(x_buf[r0:r1, :], wq_buf[s, :, c0:c1], preferred_element_type=f32)
                    store_q(q, g, lo, hi, s, c0, c1)

        def missing(us):
            names = []
            for g, s in us:
                xs = ["x%d" % i for i in range(n_x) if _X_CUTS[i] < (g + 1) * R and _X_CUTS[i + 1] > g * R]
                for name in ["w%d" % s] + xs:
                    if name not in waited:
                        waited.add(name)
                        names.append(name)
            return names

        for name in missing(units[0]):
            in_copy(name).wait()
        remaining = missing(sum(units[1:], []))

        def phase1(j, carry):
            @pl.when(j == 1)
            def _():
                for name in remaining:
                    in_copy(name).wait()

            for i in range(per_iter):
                g = _select(j, [u[i][0] for u in units])
                s = _select(j, [u[i][1] for u in units])
                q_unit(g, s, 0, R, now_rows, [] if i in _GROUP0_SLOTS else late_rows)
            return carry

        lax.fori_loop(0, _N_LOOP, phase1, 0)
        wo_copy().wait()

        o_ref = qo_scr.at[NG]
        pairs = [(h, b) for h in range(Hkv) for b in range(_GB)]

        def phase2(g, carry):
            k_copy(g).wait()
            v_copy(g).wait()
            g_next = jnp.minimum(g + 1, NG - 1)

            def scores(h, b):
                q2 = jnp.concatenate(
                    [qo_scr[g, h * rep + r, b * Sq:(b + 1) * Sq, :] for r in range(rep)], axis=0)
                return lax.dot_general(q2, k_buf[g, b, h], _NT, preferred_element_type=f32)

            def weighted_values(h, b, s):
                p = jnp.exp2(s - jnp.max(s, axis=-1, keepdims=True))
                l = jnp.sum(p, axis=-1, keepdims=True)
                o = jnp.dot(p.astype(bf16), v_buf[g, b, h], preferred_element_type=f32)
                return o, l

            def normalise(h, b, o, l):
                o = (o * pl.reciprocal(l, approx=False, full_range=False)).astype(bf16)
                for r in range(rep):
                    o_ref[h * rep + r, b * Sq:(b + 1) * Sq, :] = o[r * Sq:(r + 1) * Sq]

            def finish_late(head, e):
                s, c = divmod(head, heads_per_chunk)
                acc = q_main_scr[g_next, head, e * _VB:(e + 1) * _VB, :]
                w = wq_buf[s, DM:D, c * Dh:(c + 1) * Dh].astype(f32)
                xb = xb_scr[g_next, :, (n_now + e) * _VB:(n_now + e + 1) * _VB, :]
                for k in range(DT):
                    acc = acc + xb[k] * w[k:k + 1]
                qo_scr[g_next, head, late_rows[e]:late_rows[e] + _VB, :] = (acc * q_scale).astype(bf16)

            late_todo = [(head, e) for head in range(Hq) for e in range(n_late)]
            s_next = scores(*pairs[0])
            for _ in range(_LATE_HEAD_START):
                finish_late(*late_todo.pop(0))
            pending = None
            for i, (h, b) in enumerate(pairs):
                s_cur = s_next
                if i + 1 < len(pairs):
                    s_next = scores(*pairs[i + 1])
                cur = (h, b) + weighted_values(h, b, s_cur)
                if pending is not None:
                    normalise(*pending)
                if late_todo:
                    finish_late(*late_todo.pop(0))
                pending = cur
            normalise(*pending)
            assert not late_todo

            def o_rows(r0, nr):
                return jnp.concatenate([o_ref[h, r0:r0 + nr, :] for h in range(Hq)], axis=1)

            tail_t = lax.dot_general(wot_buf[DM:D, :], o_rows(0, R), _NT, preferred_element_type=f32)
            tail_t = jnp.concatenate([tail_t, jnp.zeros((_LANE - DT, R), f32)], axis=0)
            out_buf[g, :, DM:D] = tail_t.T[:, :DT].astype(out_buf.dtype)
            for t, (r0, nr, c0, nc) in enumerate(_OUT_PIECES):
                c1 = min(c0 + nc, DM)
                res = lax.dot_general(o_rows(r0, nr), wot_buf[c0:c1, :], _NT, preferred_element_type=f32)
                out_buf[g, r0:r0 + nr, c0:c1] = res.astype(out_buf.dtype)
                out_copy(g, t).start()
            return carry

        lax.fori_loop(0, NG, phase2, 0)
        for g in range(NG):
            for t in range(n_out):
                out_copy(g, t).wait()

    def kernel(*refs):
        def once(_, carry):
            body(*refs)
            return carry

        lax.fori_loop(0, pl.program_id(0) + 1, once, 0)

    hbm = pl.BlockSpec(memory_space=pltpu.HBM)
    out = pl.pallas_call(
        kernel,
        grid=(1,),
        in_specs=[hbm] * 7,
        out_specs=hbm,
        out_shape=jax.ShapeDtypeStruct((M, D), x.dtype),
        scratch_shapes=[
            pltpu.VMEM((M, D), bf16),
            pltpu.VMEM((n_chunks, D, _WQ_CHUNK), bf16),
            pltpu.VMEM((D, Hq * Dh), bf16),
            pltpu.VMEM((NG, _GB, Hkv, Sk, Dh), bf16),
            pltpu.VMEM((NG, _GB, Hkv, Sk, Dh), bf16),
            pltpu.VMEM((NG + 1, Hq, R, Dh), bf16),
            pltpu.VMEM((NG, R, D), bf16),
            pltpu.VMEM((NG * n_now, _VB, DT), bf16),
            pltpu.VMEM((NG * n_late, _VB, DT), bf16),
            pltpu.VMEM((NG, DT, (n_now + n_late) * _VB, _LANE), f32),
            pltpu.VMEM((NG, Hq, n_late * _VB, Dh), f32),
            pltpu.SemaphoreType.DMA((n_sems,)),
        ],
        compiler_params=pltpu.CompilerParams(
            dimension_semantics=("arbitrary",),
            vmem_limit_bytes=120 * 1024 * 1024,
            disable_semaphore_checks=True,
        ),
    )(x.reshape(M, D), x.reshape(M // _NOW[0], _NOW[0], D), x.reshape(M // _LATE[0], _LATE[0], D),
      k_cache, v_cache, wq, wo.T)
    return out.reshape(B, Sq, D)
```
